```python
import jax
import jax.numpy as jnp

def _softmax(x, axis=-1):
    return jax.nn.softmax(x, axis=axis)
def _gelu(x):
    return jax.nn.gelu(x, approximate=True)
def _silu(x):
    return jax.nn.silu(x)
def _sigmoid(x):
    return jax.nn.sigmoid(x)
def _layernorm(x, axis=-1, eps=1e-5):
    m = jnp.mean(x, axis=axis, keepdims=True)
    v = jnp.var(x, axis=axis, keepdims=True)
    return (x - m) / jnp.sqrt(v + eps)
def _scatter_add(tgt, idx, src, axis=0):
    return tgt.at[idx].add(src)
def _segment_sum(src, seg, n):
    return jax.ops.segment_sum(src, seg, n)
class _Rng:
    def __init__(self, key):
        self._k = key
    def _next(self):
        self._k, sub = jax.random.split(self._k)
        return sub
    def normal(self, shape):
        return jax.random.normal(self._next(), shape, dtype=jnp.bfloat16)
    def randint(self, lo, hi, shape):
        return jax.random.randint(self._next(), shape, lo, hi, dtype=jnp.int32)
    def uniform(self, shape, lo=0.0, hi=1.0):
        return jax.random.uniform(self._next(), shape, jnp.bfloat16, lo, hi)
    def permutation(self, n):
        return jax.random.permutation(self._next(), n)


kernel_name = 'concat_heads__ssm_conv_h3__compressed_kv_cla__prompt'

def setup_inputs():
    _rng = _Rng(jax.random.key(int.from_bytes(__import__("os").urandom(4), "little")))
    _w = (lambda a: (lambda t: t.astype(jnp.bfloat16) if jnp.issubdtype(t.dtype, jnp.floating) else t)(jnp.asarray(a)))
    def _A_setup():
        B, S, D = 1, 2048, 448
        ks = 4
        return {
            "q": _w((lambda *s: _rng.normal(s) * 0.05)(B, S, D)),
            "k": _w((lambda *s: _rng.normal(s) * 0.05)(B, S, D)),
            "v": _w((lambda *s: _rng.normal(s) * 0.05)(B, S, D)),
            "shift_k": _w((lambda *s: _rng.normal(s) * 0.05)(D, ks) * 0.5),
            "ssm_k": _w((lambda *s: _rng.normal(s) * 0.05)(D, S) * (1.0 / S ** 0.5)),
            "ssm_D": _w((lambda *s: _rng.normal(s) * 0.05)(D)),
        }
    _A_in = _A_setup()

    def _B_setup():
        B, H, Sq, Sk, D, M = 1, 16, 2048, 2048, 256, 448
        Dc = 4 * D
        return {
            "x": _w((lambda *s: _rng.normal(s) * 0.05)(B, Sq, M)),
            "c_kv": _w((lambda *s: _rng.normal(s) * 0.05)(B, Sk, Dc)),
            "w_q": _w((lambda *s: _rng.normal(s) * 0.05)(M, H, D) * (M ** -0.5)),
            "w_uk": _w((lambda *s: _rng.normal(s) * 0.05)(Dc, H, D) * (Dc ** -0.5)),
            "w_uv": _w((lambda *s: _rng.normal(s) * 0.05)(Dc, H, D) * (Dc ** -0.5)),
            "w_o": _w((lambda *s: _rng.normal(s) * 0.05)(H, D, M) * ((H * D) ** -0.5)),
        }
    _B_in = _B_setup()

    return {
        "A_q": _A_in["q"],
        "A_k": _A_in["k"],
        "A_v": _A_in["v"],
        "A_shift_k": _A_in["shift_k"],
        "A_ssm_k": _A_in["ssm_k"],
        "A_ssm_D": _A_in["ssm_D"],
        "B_x": _B_in["x"],
        "B_c_kv": _B_in["c_kv"],
        "B_w_q": _B_in["w_q"],
        "B_w_uk": _B_in["w_uk"],
        "B_w_uv": _B_in["w_uv"],
        "B_w_o": _B_in["w_o"],
    }

def reference(A_q, A_k, A_v, A_shift_k, A_ssm_k, A_ssm_D, B_x, B_c_kv, B_w_q, B_w_uk, B_w_uv, B_w_o):
    def _A_ref(q, k, v, shift_k, ssm_k, ssm_D):
        B, S, D = q.shape
        ks = shift_k.shape[-1]
        k_pad = jnp.pad(k, ((0, 0), (ks - 1, 0), (0, 0)))
        k_shift = jnp.zeros_like(k)
        for t in range(ks):
            k_shift = k_shift + k_pad[:, t:t + S, :] * shift_k[:, ks - 1 - t][None, None, :]
        kv = k_shift * v
        L = 2 * S
        kv_pad = jnp.pad(kv, ((0, 0), (0, S), (0, 0)))
        kf_pad = jnp.pad(ssm_k, ((0, 0), (0, S)))
        kv_f = (lambda x, axes=(-2,-1): jnp.fft.rfft2(x.astype(jnp.float32), axes=axes))(kv_pad[:, None, :, :], axes=(1, 2))
        kf_f = (lambda x, axes=(-2,-1): jnp.fft.rfft2(x.astype(jnp.float32), axes=axes))(kf_pad[:, None, :], axes=(1, 2))
        kf_f = (lambda x, *d: x.transpose(*d))(kf_f, 1, 2, 0)
        y_f = kv_f * kf_f[None, :, :, :]
        y = (lambda x, s, axes=(-2,-1): jnp.fft.irfft2(x, s=s, axes=axes).astype(jnp.bfloat16))(y_f, (1, L), axes=(1, 2))[:, 0, :S, :]
        y = y + kv * ssm_D[None, None, :]
        return q * y

    def _B_ref(x, c_kv, w_q, w_uk, w_uv, w_o):
        B, Sq, M = x.shape[0], x.shape[1], x.shape[2]
        Sk = c_kv.shape[1]
        H, D = w_q.shape[1], w_q.shape[2]
        q = jnp.einsum("bqm,mhd->bhqd", x, w_q)
        k = jnp.einsum("bkc,chd->bhkd", c_kv, w_uk)
        v = jnp.einsum("bkc,chd->bhkd", c_kv, w_uv)
        scores = jnp.einsum("bhqd,bhkd->bhqk", q, k) * (D ** -0.5)
        off = Sk - Sq
        qi = jnp.arange(Sq)[:, None]
        kj = jnp.arange(Sk)[None, :]
        cmask = kj <= (qi + off)
        scores = jnp.where(cmask[None, None], scores, -1e9)
        p = _softmax(scores, axis=-1)
        ctx = jnp.einsum("bhqk,bhkd->bhqd", p, v)
        return jnp.einsum("bhqd,hdm->bqm", ctx, w_o)

    a = _A_ref(A_q, A_k, A_v, A_shift_k, A_ssm_k, A_ssm_D)
    b = _B_ref(B_x, B_c_kv, B_w_q, B_w_uk, B_w_uv, B_w_o)
    return jnp.concatenate([a, b], axis=-1)
```

```python
import functools
import numpy as np
import jax
import jax.numpy as jnp
from jax import lax
import jax.experimental.pallas as pl
import jax.experimental.pallas.tpu as pltpu

S = 2048
DA = 448
H = 16
D = 256
DC = 1024
T = 256
NCH = S // T
TQ = 256
DO_A = True
DO_B = True
LOG2E = 1.4426950408889634
bf16 = jnp.bfloat16
f32 = jnp.float32


def _dft_mats():
    f = np.arange(T, dtype=np.float64)[None, :]
    j = np.arange(T, dtype=np.float64)[:, None]
    ang = np.pi * (((2 * f + 1) * j) % (4 * T)) / (2 * T)
    F = np.concatenate([np.cos(ang), -np.sin(ang)], axis=1)
    G = F.T / T
    return F.astype(bf16), np.ascontiguousarray(G).astype(bf16)


def _nt(a, b):
    return lax.dot_general(a, b, (((1,), (1,)), ((), ())), preferred_element_type=f32)


def _nn(a, b):
    return jnp.dot(a, b, preferred_element_type=f32)


def _head_weights(h, items):
    sh = (16 * (1 - (h & 1))).astype(jnp.uint32)
    for j in range(H // 2):
        @pl.when((h >> 1) == j)
        def _():
            for w_ref, dst in items:
                for ct in range(2):
                    w = w_ref.at[ct].bitcast(jnp.uint32)[pl.ds(j, dst.shape[0], stride=H // 2), :]
                    w = (w << sh) & jnp.uint32(0xFFFF0000)
                    dst[:, pl.ds(ct * 128, 128)] = pltpu.bitcast(w, f32).astype(bf16)


def _conv_phase(q_ref, k_ref, v_ref, sh_ref, d_ref, sk_ref, F_ref, G_ref,
                u_scr, U_scr, K_scr, Z_scr, out_ref):
    par = jnp.concatenate([sh_ref[...].astype(f32), d_ref[...].astype(f32),
                           jnp.zeros((3, DA), f32)], axis=0)
    U_scr[0, 0:8, 0:DA] = par
    par = U_scr[0, 0:128, 0:512].T
    RB = 64
    lane = lax.broadcasted_iota(jnp.int32, (RB, S), 1)
    for r in range(DA // RB):
        rows = pl.ds(r * RB, RB)
        kc = k_ref[rows, :].astype(f32)
        pr = par[r * RB:(r + 1) * RB]
        acc = kc * pr[:, 0:1]
        for j in range(1, 4):
            acc = acc + jnp.where(lane >= j, pltpu.roll(kc, j, 1), 0.0) * pr[:, j:j + 1]
        u_scr[rows, :] = (acc * v_ref[rows, :].astype(f32)).astype(bf16)
    for c in range(NCH):
        cols = pl.ds(c * T, T)
        U_scr[c] = _nn(u_scr[:, cols], F_ref[...])
        K_scr[c] = _nn(sk_ref[:, cols], F_ref[...])

    R = 16
    sgn = (1 - 2 * (lax.broadcasted_iota(jnp.int32, (R, T), 1) % 2)).astype(f32)
    re = pl.ds(0, T)
    im = pl.ds(T, T)

    def zbody(i, _):
        rows = pl.ds(pl.multiple_of(i * R, R), R)
        kr = [K_scr[0, rows, re]]
        ki = [K_scr[0, rows, im]]
        for m in range(1, NCH):
            kr.append(K_scr[m, rows, re] - sgn * K_scr[m - 1, rows, im])
            ki.append(K_scr[m, rows, im] + sgn * K_scr[m - 1, rows, re])
        for c in range(NCH):
            zr = zi = None
            for m in range(c + 1):
                ur = U_scr[c - m, rows, re]
                ui = U_scr[c - m, rows, im]
                tr = kr[m] * ur - ki[m] * ui
                ti = kr[m] * ui + ki[m] * ur
                zr = tr if zr is None else zr + tr
                zi = ti if zi is None else zi + ti
            Z_scr[c, rows, re] = zr.astype(bf16)
            Z_scr[c, rows, im] = zi.astype(bf16)
        return None

    lax.fori_loop(0, DA // R, zbody, None)
    dcol = par[0:DA, 4:5]
    for c in range(NCH):
        cols = pl.ds(c * T, T)
        y = _nn(Z_scr[c], G_ref[...])
        y = y + u_scr[:, cols].astype(f32) * dcol
        a = q_ref[:, cols].astype(f32) * y
        out_ref[cols, 0:DA] = a.T.astype(bf16)


def _kernel(q_ref, k_ref, v_ref, sh_ref, sk_ref, d_ref, F_ref, G_ref,
            x_hbm, c_hbm, wq_hbm, wuk_hbm, wuv_hbm, wo_hbm, out_ref,
            u_scr, U_scr, K_scr, Z_scr,
            xt_scr, x_scr, c_scr, wq_scr, wuk_scr, wuv_scr, wo_scr, wq_h, wuk_h, wuv_h, qh, kh, vh, ctx, acc, sems):
    pairs = [(x_hbm, xt_scr), (c_hbm, c_scr)]
    for s, d in [(wq_hbm, wq_scr), (wuk_hbm, wuk_scr), (wuv_hbm, wuv_scr)]:
        for ct in range(2):
            pairs.append((s.at[:, pl.ds(ct * 128, 128)], d.at[ct]))
    pairs.append((wo_hbm, wo_scr.at[:, pl.ds(64, DA), :]))
    copies = [pltpu.make_async_copy(s, d, sems.at[i]) for i, (s, d) in enumerate(pairs)]

    for cp in copies:
        cp.start()
    if DO_A:
        _conv_phase(q_ref, k_ref, v_ref, sh_ref, d_ref, sk_ref, F_ref, G_ref,
                    u_scr, U_scr, K_scr, Z_scr, out_ref)
    acc[...] = jnp.zeros_like(acc)
    wo_scr[:, 0:64, :] = jnp.zeros((H, 64, D), bf16)
    copies[0].wait()
    for c in range(NCH):
        x_scr[pl.ds(c * T, T), :] = xt_scr[:, pl.ds(c * T, T)].T
    for cp in copies[1:]:
        cp.wait()

    def head(h, _):
        _head_weights(h, [(wq_scr, wq_h), (wuk_scr, wuk_h), (wuv_scr, wuv_h)])
        qh[...] = (_nn(x_scr[...], wq_h[...]) * (LOG2E * D ** -0.5)).astype(bf16)
        kh[...] = _nn(c_scr[...], wuk_h[...]).astype(bf16)
        vh[...] = _nn(c_scr[...], wuv_h[...]).astype(bf16)
        mask = lax.broadcasted_iota(jnp.int32, (TQ, TQ), 1) <= lax.broadcasted_iota(jnp.int32, (TQ, TQ), 0)
        for i in range(S // TQ):
            rows = pl.ds(i * TQ, TQ)
            n = i * TQ
            q = qh[rows, :]
            sd = jnp.where(mask, _nt(q, kh[rows, :]), -1e9)
            m = jnp.max(sd, axis=1, keepdims=True)
            if i > 0:
                s = _nt(q, kh[0:n, :])
                m = jnp.maximum(m, jnp.max(s, axis=1, keepdims=True))
            pd = jnp.exp2(sd - m)
            l = jnp.sum(pd, axis=1, keepdims=True)
            o = _nn(pd.astype(bf16), vh[rows, :])
            if i > 0:
                p = jnp.exp2(s - m)
                l = l + jnp.sum(p, axis=1, keepdims=True)
                o = o + _nn(p.astype(bf16), vh[0:n, :])
            ctx[rows, :] = (o * (1.0 / l)).astype(bf16)
        acc[...] += _nt(ctx[...], wo_scr[h])

    if DO_B:
        lax.fori_loop(0, H, head, None)
    lane = lax.broadcasted_iota(jnp.int32, (S, 128), 1)
    out_ref[:, 384:512] = jnp.where(lane < 64, out_ref[:, 384:512], acc[:, 0:128].astype(bf16))
    out_ref[:, 512:896] = acc[:, 128:512].astype(bf16)


@jax.jit
def pallas_concat_heads__ssm_conv_h3__compressed_kv_cla__prompt_kernel(
    A_q, A_k, A_v, A_shift_k, A_ssm_k, A_ssm_D, B_x, B_c_kv, B_w_q, B_w_uk, B_w_uv, B_w_o,
):
    F, G = _dft_mats()

    def whole(shape):
        return pl.BlockSpec(shape, lambda h: (0,) * len(shape), pipeline_mode=pl.Buffered(1))

    def tr(a):
        return a.reshape(S, DA).T

    hbm = pl.BlockSpec(memory_space=pl.ANY)
    out = pl.pallas_call(
        _kernel,
        grid=(1,),
        in_specs=[whole((DA, S))] * 3 + [whole((4, DA)), whole((DA, S)), whole((1, DA)),
                                         whole((T, 2 * T)), whole((2 * T, T)),
                                         hbm, hbm, hbm, hbm, hbm, hbm],
        out_specs=pl.BlockSpec((S, 2 * DA), lambda h: (0, 0)),
        out_shape=jax.ShapeDtypeStruct((S, 2 * DA), bf16),
        scratch_shapes=[
            pltpu.VMEM((DA, S), bf16), pltpu.VMEM((NCH, DA, 2 * T), f32),
            pltpu.VMEM((NCH, DA, 2 * T), f32), pltpu.VMEM((NCH, DA, 2 * T), bf16),
            pltpu.VMEM((DA, S), bf16), pltpu.VMEM((S, DA), bf16), pltpu.VMEM((S, DC), bf16),
            pltpu.VMEM((2, DA * H, 128), bf16), pltpu.VMEM((2, DC * H, 128), bf16), pltpu.VMEM((2, DC * H, 128), bf16),
            pltpu.VMEM((H, 512, D), bf16),
            pltpu.VMEM((DA, D), bf16), pltpu.VMEM((DC, D), bf16), pltpu.VMEM((DC, D), bf16),
            pltpu.VMEM((S, D), bf16), pltpu.VMEM((S, D), bf16), pltpu.VMEM((S, D), bf16),
            pltpu.VMEM((S, D), bf16), pltpu.VMEM((S, 512), f32),
            pltpu.SemaphoreType.DMA((9,)),
        ],
        compiler_params=pltpu.CompilerParams(
            dimension_semantics=("arbitrary",), vmem_limit_bytes=110 * 1024 * 1024),
    )(tr(A_q), tr(A_k), tr(A_v), A_shift_k.T, A_ssm_k,
      A_ssm_D.reshape(1, DA), F, G,
      tr(B_x), B_c_kv.reshape(S, DC), B_w_q.reshape(DA * H, D),
      B_w_uk.reshape(DC * H, D), B_w_uv.reshape(DC * H, D), B_w_o.transpose(0, 2, 1))
    return out.reshape(1, S, 2 * DA)
```
